```python
import os as _os
_os.environ.setdefault("JAX_PLATFORMS", "cpu")
import jax
import jax.numpy as jnp

def _softmax(x, axis=-1):
    return jax.nn.softmax(x, axis=axis)
def _gelu(x):
    return jax.nn.gelu(x, approximate=True)
def _silu(x):
    return jax.nn.silu(x)
def _sigmoid(x):
    return jax.nn.sigmoid(x)
def _layernorm(x, axis=-1, eps=1e-5):
    m = jnp.mean(x, axis=axis, keepdims=True)
    v = jnp.var(x, axis=axis, keepdims=True)
    return (x - m) / jnp.sqrt(v + eps)
def _scatter_add(tgt, idx, src, axis=0):
    return tgt.at[idx].add(src)
def _segment_sum(src, seg, n):
    return jax.ops.segment_sum(src, seg, n)
class _Rng:
    def __init__(self, key):
        self._k = key
    def _next(self):
        self._k, sub = jax.random.split(self._k)
        return sub
    def normal(self, shape):
        return jax.random.normal(self._next(), shape, dtype=jnp.bfloat16)
    def randint(self, lo, hi, shape):
        return jax.random.randint(self._next(), shape, lo, hi, dtype=jnp.int32)
    def uniform(self, shape, lo=0.0, hi=1.0):
        return jax.random.uniform(self._next(), shape, jnp.bfloat16, lo, hi)
    def permutation(self, n):
        return jax.random.permutation(self._next(), n)


kernel_name = 'gated_mix__mha_block__mha_block__prompt'

def setup_inputs():
    _rng = _Rng(jax.random.key(int.from_bytes(__import__("os").urandom(4), "little")))
    _w = (lambda a: (lambda t: t.astype(jnp.bfloat16) if jnp.issubdtype(t.dtype, jnp.floating) else t)(jnp.asarray(a)))
    def _A_setup():
        B, S, D, H = 1, 2048, 448, 16
        return {
            "x": _w((lambda *s: _rng.normal(s) * 0.05)(B, S, D)),
            "wqkv": _w((lambda *s: _rng.normal(s) * 0.4)(D, 3 * D)),
            "wo": _w((lambda *s: _rng.normal(s) * 0.05)(D, D)),
        }
    _A_in = _A_setup()

    def _B_setup():
        B, S, D, H = 1, 2048, 448, 16
        return {
            "x": _w((lambda *s: _rng.normal(s) * 0.05)(B, S, D)),
            "wqkv": _w((lambda *s: _rng.normal(s) * 0.4)(D, 3 * D)),
            "wo": _w((lambda *s: _rng.normal(s) * 0.05)(D, D)),
        }
    _B_in = _B_setup()

    return {
        "A_x": _A_in["x"],
        "A_wqkv": _A_in["wqkv"],
        "A_wo": _A_in["wo"],
        "B_x": _B_in["x"],
        "B_wqkv": _B_in["wqkv"],
        "B_wo": _B_in["wo"],
        "gate_w": _w((lambda *s: _rng.normal(s) * 0.05)(448) * 16.0),
    }

def reference(A_x, A_wqkv, A_wo, B_x, B_wqkv, B_wo, gate_w):
    def _A_ref(x, wqkv, wo):
        B, S, D = x.shape
        H = 16
        Dh = D // H
        qkv = (lambda x, *d: x.transpose(*d))((x @ wqkv).reshape(B, S, 3, H, Dh), 2, 0, 3, 1, 4)
        q, k, v = qkv[0], qkv[1], qkv[2]
        scores = jnp.einsum("bhqd,bhkd->bhqk", q, k) * (Dh ** -0.5)
        p = _softmax(scores, axis=-1)
        o = jnp.einsum("bhqk,bhkd->bhqd", p, v)
        return (lambda x, *d: x.transpose(*d))(o, 0, 2, 1, 3).reshape(B, S, D) @ wo

    def _B_ref(x, wqkv, wo):
        B, S, D = x.shape
        H = 16
        Dh = D // H
        qkv = (lambda x, *d: x.transpose(*d))((x @ wqkv).reshape(B, S, 3, H, Dh), 2, 0, 3, 1, 4)
        q, k, v = qkv[0], qkv[1], qkv[2]
        scores = jnp.einsum("bhqd,bhkd->bhqk", q, k) * (Dh ** -0.5)
        p = _softmax(scores, axis=-1)
        o = jnp.einsum("bhqk,bhkd->bhqd", p, v)
        return (lambda x, *d: x.transpose(*d))(o, 0, 2, 1, 3).reshape(B, S, D) @ wo

    x = A_x
    g = _sigmoid((x * gate_w).sum(-1, keepdims=True))
    a = _A_ref(x, A_wqkv, A_wo)
    b = _B_ref(x, B_wqkv, B_wo)
    return g * a + (1 - g) * b
```

```python
import jax
import jax.numpy as jnp
import numpy as np
import jax.experimental.pallas as pl
import jax.experimental.pallas.tpu as pltpu

f32, bf16 = jnp.float32, jnp.bfloat16
S, D, H = 2048, 448, 16
DH = D // H
DP = 32
HP = H * DP
PC = 512
NC = S // PC
PQ, PK, QV_MERGE, K_NN = 512, 512, True, False
GR = 16
NN = (((1,), (0,)), ((), ()))
NT = (((1,), (1,)), ((), ()))
QSCALE = float(DH ** -0.5 * np.log2(np.e))
SAFE_LOG2 = 50.0


def _pad_heads(a, fill):
    blocks = []
    for h in range(H):
        blocks += [a[h * DH:(h + 1) * DH, :], fill]
    return jnp.concatenate(blocks, axis=0)


def _kernel(x_hbm, aw_hbm, awo_hbm, bw_hbm, bwo_hbm, gw_hbm, out_hbm,
            gw_ref, x_buf, xn_s, w_buf, wo_buf, wt_s, wqv_s, wk_s, k_s, qT_s, vT_s, woT_s, oT_s, qm_s, acc_s, g_s,
            out_buf, in_sems, out_sems):
    x_cp = [pltpu.make_async_copy(x_hbm.at[:, pl.ds(c * PC, PC)], x_buf.at[:, pl.ds(c * PC, PC)], in_sems.at[c])
            for c in range(NC)]
    w_cp = [pltpu.make_async_copy(src, w_buf.at[i], in_sems.at[NC + i])
            for i, src in enumerate((aw_hbm, bw_hbm))]
    wo_cp = [pltpu.make_async_copy(src, wo_buf.at[pl.ds(i * D, D)], in_sems.at[NC + 2 + i])
             for i, src in enumerate((awo_hbm, bwo_hbm))]

    gw_cp = pltpu.make_async_copy(gw_hbm, gw_ref, in_sems.at[NC + 4])

    def prep_wqkv(br):
        wt_s[br] = w_buf[br].astype(f32).T
        wqv_s[br, 0:D, :] = wt_s[br, 0:D, :].astype(bf16)
        wqv_s[br, D:2 * D, :] = wt_s[br, 2 * D:3 * D, :].astype(bf16)
        wkp = _pad_heads(wt_s.at[br, D:2 * D], jnp.zeros((DP - DH, D), f32))
        if K_NN:
            wk_s[br] = wkp.T.astype(bf16)
        else:
            wk_s[br] = wkp.astype(bf16)

    def prep_wo(br):
        if br == 1:
            woT_s[...] = wo_buf[...].astype(f32).T.astype(bf16)

    def x_cols(c0, n):
        return x_buf[:, pl.ds(c0, n)]

    def proj_qv(br, c0, n):
        cols = pl.ds(c0, n)
        xT = x_cols(c0, n)
        if QV_MERGE:
            qv = jax.lax.dot_general(wqv_s[br], xT, NN, preferred_element_type=f32)
            qT, vT = qv[0:D], qv[D:2 * D]
        else:
            qT = jax.lax.dot_general(wqv_s[br, 0:D, :], xT, NN, preferred_element_type=f32)
            vT = jax.lax.dot_general(wqv_s[br, D:2 * D, :], xT, NN, preferred_element_type=f32)
        qT = _pad_heads(qT * QSCALE, jnp.zeros((DP - DH, n), f32)).astype(bf16)
        qT_s[br * HP:(br + 1) * HP, cols] = qT
        ones_row = (jax.lax.broadcasted_iota(jnp.int32, (DP - DH, n), 0) == 0).astype(f32)
        vT_s[br * HP:(br + 1) * HP, cols] = _pad_heads(vT, ones_row).astype(bf16)
        q_l1 = jnp.sum(jnp.abs(qT.astype(f32)).reshape(H, DP, n), axis=1)
        return q_l1

    def proj_k(br, c0, n):
        cols = pl.ds(c0, n)
        if br == 0:
            xT = x_cols(c0, n)
            xn_s[cols, :] = xT.astype(f32).T.astype(bf16)
            z = jax.lax.dot_general(jnp.broadcast_to(gw_ref[...].reshape(1, D), (GR, D)), xT, NN,
                                    preferred_element_type=f32)
            g_s[:, cols] = jax.nn.sigmoid(z[0:8, :])
        k = jax.lax.dot_general(xn_s[cols, :], wk_s[br], NN if K_NN else NT,
                                preferred_element_type=f32).astype(bf16)
        k_s[br, cols, :] = k
        k_max = jnp.max(jnp.abs(k.astype(f32)).reshape(n // 8, 8, HP), axis=0)
        return k_max

    w_cp[0].start()
    x_cp[0].start()
    gw_cp.start()
    w_cp[0].wait()
    for cp in x_cp[1:] + w_cp[1:] + wo_cp:
        cp.start()
    prep_wqkv(0)
    arrivals = {0: [x_cp[0], gw_cp], 1: x_cp[1:2], 2: x_cp[2:] + w_cp[1:] + wo_cp}
    stats = [[[], []], [[], []]]
    for br in range(2):
        for c in range(NC):
            if br == 0:
                for cp in arrivals.get(c, []):
                    cp.wait()
            stats[br][0].append(proj_qv(br, c * PC, PC))
            stats[br][1].append(proj_k(br, c * PC, PC))
            if br == 0 and c == 2:
                prep_wqkv(1)
            if br == 1 and c < 2:
                prep_wo(c)
    bounds = []
    for br in range(2):
        q_l1 = _reduce(jnp.maximum, stats[br][0])
        k_max = _reduce(jnp.maximum, stats[br][1])
        bounds.append(jnp.max(q_l1) * jnp.max(k_max))
    safe = jnp.logical_and(bounds[0] <= SAFE_LOG2, bounds[1] <= SAFE_LOG2)

    g_row = g_s[0:1, :]

    def masked_q(i):
        grp = pl.multiple_of((i // 4) * 128, 128)
        qg = qT_s[pl.ds(grp, 128), :]
        row = jax.lax.broadcasted_iota(jnp.int32, (128, S), 0)
        qm_s[...] = jnp.where((row >> 5) == (i % 4), qg, jnp.zeros_like(qg))

    def finalize(i):
        acc = acc_s[...]
        gate = jnp.where(i < H, g_row, 1.0 - g_row)
        o = acc * (gate / acc[DH:DH + 1, :])
        oT_s[pl.ds(pl.multiple_of(i * DP, DP), DP), :] = o.astype(bf16)

    def attend(use_max):
        def head(i, carry):
            grp = pl.multiple_of(((i % H) // 4) * 128, 128)
            s = jax.lax.dot_general(k_s[i // H, :, pl.ds(grp, 128)], qm_s[...], NN,
                                    preferred_element_type=f32)
            finalize(jnp.where(i == 0, 2 * H, i - 1))
            if use_max:
                s = s - jnp.max(s, axis=0, keepdims=True)
            p = jnp.exp2(s).astype(bf16)
            vT = vT_s[pl.ds(pl.multiple_of(i * DP, DP), DP), :]
            acc = jax.lax.dot_general(vT, p, NN, preferred_element_type=f32)
            masked_q(jnp.minimum(i + 1, 2 * H - 1))
            acc_s[...] = acc
            return carry
        jax.lax.fori_loop(0, 2 * H, head, 0)

    masked_q(jnp.int32(0))
    acc_s[...] = jnp.ones((DP, S), f32)

    @pl.when(safe)
    def _fast():
        attend(False)

    @pl.when(jnp.logical_not(safe))
    def _exact_max():
        attend(True)

    finalize(jnp.int32(2 * H - 1))

    out_cp = []
    for c in range(NC):
        cols = pl.ds(c * PC, PC)
        o = oT_s[0:2 * HP, cols].astype(f32)
        o = jnp.concatenate([o[i * DP:i * DP + DH, :] for i in range(2 * H)], axis=0).astype(bf16)
        outT = jax.lax.dot_general(woT_s[...], o, NN, preferred_element_type=f32)
        out_buf[c] = outT.astype(bf16)
        cp = pltpu.make_async_copy(out_buf.at[c], out_hbm.at[:, cols], out_sems.at[c])
        cp.start()
        out_cp.append(cp)
    for cp in out_cp:
        cp.wait()


def _reduce(fn, xs):
    acc = xs[0]
    for x in xs[1:]:
        acc = fn(acc, x)
    return acc


@jax.jit
def pallas_gated_mix__mha_block__mha_block__prompt_kernel(
    A_x: jax.Array,
    A_wqkv: jax.Array,
    A_wo: jax.Array,
    B_x: jax.Array,
    B_wqkv: jax.Array,
    B_wo: jax.Array,
    gate_w: jax.Array,
):
    del B_x
    hbm = pl.BlockSpec(memory_space=pltpu.HBM)
    outT = pl.pallas_call(
        _kernel,
        in_specs=[hbm] * 6,
        out_specs=hbm,
        out_shape=jax.ShapeDtypeStruct((D, S), bf16),
        scratch_shapes=[
            pltpu.VMEM((D,), bf16),
            pltpu.VMEM((D, S), bf16),
            pltpu.VMEM((S, D), bf16),
            pltpu.VMEM((2, D, 3 * D), bf16),
            pltpu.VMEM((2 * D, D), bf16),
            pltpu.VMEM((2, 3 * D, D), f32),
            pltpu.VMEM((2, 2 * D, D), bf16),
            pltpu.VMEM((2, D, HP) if K_NN else (2, HP, D), bf16),
            pltpu.VMEM((2, S, HP), bf16),
            pltpu.VMEM((2 * HP, S), bf16),
            pltpu.VMEM((2 * HP, S), bf16),
            pltpu.VMEM((D, 2 * D), bf16),
            pltpu.VMEM((2 * HP + DP, S), bf16),
            pltpu.VMEM((128, S), bf16),
            pltpu.VMEM((DP, S), f32),
            pltpu.VMEM((8, S), f32),
            pltpu.VMEM((NC, D, PC), bf16),
            pltpu.SemaphoreType.DMA((NC + 5,)),
            pltpu.SemaphoreType.DMA((NC,)),
        ],
        compiler_params=pltpu.CompilerParams(vmem_limit_bytes=100 * 1024 * 1024),
    )(A_x.reshape(S, D).T, A_wqkv, A_wo, B_wqkv, B_wo, gate_w)
    return outT.T.reshape(1, S, D)
```

```python
import jax
import jax.numpy as jnp
import numpy as np
import jax.experimental.pallas as pl
import jax.experimental.pallas.tpu as pltpu

f32, bf16 = jnp.float32, jnp.bfloat16
S, D, H = 2048, 448, 16
DH = D // H
DP = 32
HP = H * DP
PC = 512
NC = S // PC
OUT_CHUNKS = ((0, 512), (512, 512), (1024, 512), (1536, 256), (1792, 256))
GR = 16
NN = (((1,), (0,)), ((), ()))
NT = (((1,), (1,)), ((), ()))
QSCALE = float(DH ** -0.5 * np.log2(np.e))
V_RANGE = 2.0 ** 60
SAFE_LOG2 = 50.0


def _pad_heads(a, fill):
    blocks = []
    for h in range(H):
        blocks += [a[h * DH:(h + 1) * DH, :], fill]
    return jnp.concatenate(blocks, axis=0)


def _kernel(x_hbm, aw_hbm, awo_hbm, bw_hbm, bwo_hbm, gw_hbm, out_hbm,
            gw_ref, x_buf, xn_s, w_buf, wo_buf, wt_s, wqv_s, wk_s, k_s, qT_s, vT_s, woT_s, oT_s, qm_s, acc_s, g_s,
            out_buf, in_sems, out_sems, aw_sems):
    x_cp = [pltpu.make_async_copy(x_hbm.at[:, pl.ds(c * PC, PC)], x_buf.at[:, pl.ds(c * PC, PC)], in_sems.at[c])
            for c in range(NC)]
    bw_cp = pltpu.make_async_copy(bw_hbm, w_buf.at[1], in_sems.at[NC])
    wo_cp = [pltpu.make_async_copy(src, wo_buf.at[pl.ds(i * D, D)], in_sems.at[NC + 1 + i])
             for i, src in enumerate((awo_hbm, bwo_hbm))]

    aw_parts = [pltpu.make_async_copy(aw_hbm.at[:, pl.ds(a, n)], w_buf.at[0, :, pl.ds(a, n)], aw_sems.at[j])
                for j, (a, n) in enumerate(((384, 512), (896, 448), (0, 384)))]
    gw_cp = pltpu.make_async_copy(gw_hbm, gw_ref, in_sems.at[NC + 3])

    def prep_wqkv(br):
        wt_s[br] = w_buf[br].astype(f32).T
        wqv_s[br, 0:D, :] = wt_s[br, 0:D, :].astype(bf16)
        wqv_s[br, D:2 * D, :] = wt_s[br, 2 * D:3 * D, :].astype(bf16)
        wkp = _pad_heads(wt_s.at[br, D:2 * D], jnp.zeros((DP - DH, D), f32))
        wk_s[br] = wkp.astype(bf16)

    def proj_qv(br, c0, n):
        cols = pl.ds(c0, n)
        xT = x_buf[:, cols]
        qv = jax.lax.dot_general(wqv_s[br], xT, NN, preferred_element_type=f32)
        qT, vT = qv[0:D], qv[D:2 * D]
        qT = _pad_heads(qT * QSCALE, jnp.zeros((DP - DH, n), f32)).astype(bf16)
        qT_s[br * HP:(br + 1) * HP, cols] = qT
        ones_row = (jax.lax.broadcasted_iota(jnp.int32, (DP - DH, n), 0) == 0).astype(f32)
        vT_s[br * HP:(br + 1) * HP, cols] = _pad_heads(vT, ones_row).astype(bf16)
        v_max = jnp.max(jnp.abs(vT).reshape(D // 8, 8, n), axis=0)
        q_l1 = jnp.sum(jnp.abs(qT.astype(f32)).reshape(H, DP, n), axis=1)
        return q_l1, v_max

    def proj_k(br, c0, n):
        cols = pl.ds(c0, n)
        if br == 0:
            xT = x_buf[:, cols]
            xn_s[cols, :] = xT.astype(f32).T.astype(bf16)
            z = jax.lax.dot_general(jnp.broadcast_to(gw_ref[...].reshape(1, D), (GR, D)), xT, NN,
                                    preferred_element_type=f32)
            g_s[:, cols] = jax.nn.sigmoid(z[0:8, :])
        k = jax.lax.dot_general(xn_s[cols, :], wk_s[br], NT,
                                preferred_element_type=f32).astype(bf16)
        k_s[br, cols, :] = k
        k_max = jnp.max(jnp.abs(k.astype(f32)).reshape(n // 8, 8, HP), axis=0)
        return k_max

    aw_parts[0].start()
    x_cp[0].start()
    gw_cp.start()
    aw_parts[0].wait()
    aw_parts[1].start()
    aw_parts[2].start()
    x_cp[0].wait()
    gw_cp.wait()
    for cp in x_cp[1:] + [bw_cp] + wo_cp:
        cp.start()
    wt_s[0, 384:896, :] = w_buf[0, :, 384:896].astype(f32).T
    wk_s[0] = _pad_heads(wt_s.at[0, D:2 * D], jnp.zeros((DP - DH, D), f32)).astype(bf16)
    kstat0 = proj_k(0, 0, PC)
    aw_parts[1].wait()
    aw_parts[2].wait()
    wt_s[0, 0:384, :] = w_buf[0, :, 0:384].astype(f32).T
    wt_s[0, 896:1344, :] = w_buf[0, :, 896:1344].astype(f32).T
    wqv_s[0, 0:D, :] = wt_s[0, 0:D, :].astype(bf16)
    wqv_s[0, D:2 * D, :] = wt_s[0, 2 * D:3 * D, :].astype(bf16)
    arrivals = {1: x_cp[1:2], 2: x_cp[2:] + [bw_cp] + wo_cp}
    stats = [[[], []], [[], []]]
    for br in range(2):
        for c in range(NC):
            if br == 0:
                for cp in arrivals.get(c, []):
                    cp.wait()
            stats[br][0].append(proj_qv(br, c * PC, PC))
            stats[br][1].append(kstat0 if (br, c) == (0, 0) else proj_k(br, c * PC, PC))
            if br == 0 and c == 2:
                prep_wqkv(1)
            if br == 1 and c == 1:
                woT_s[...] = wo_buf[...].astype(f32).T.astype(bf16)
    bounds = []
    for br in range(2):
        q_l1 = _reduce(jnp.maximum, [t[0] for t in stats[br][0]])
        v_max = jnp.max(_reduce(jnp.maximum, [t[1] for t in stats[br][0]]))
        k_max = _reduce(jnp.maximum, stats[br][1])
        score_bound = jnp.max(q_l1) * jnp.max(k_max)
        bounds.append(jnp.logical_and(score_bound <= SAFE_LOG2,
                                      jnp.logical_and(v_max <= V_RANGE, v_max >= 1.0 / V_RANGE)))
    safe = jnp.logical_and(bounds[0], bounds[1])

    g_row = g_s[0:1, :]

    def masked_q(i):
        grp = pl.multiple_of((i // 4) * 128, 128)
        qg = qT_s[pl.ds(grp, 128), :]
        row = jax.lax.broadcasted_iota(jnp.int32, (128, S), 0)
        qm_s[...] = jnp.where((row >> 5) == (i % 4), qg, jnp.zeros_like(qg))

    def finalize(i):
        acc = acc_s[...]
        gate = jnp.where(i < H, g_row, 1.0 - g_row)
        o = acc * (gate / acc[DH:DH + 1, :])
        oT_s[pl.ds(pl.multiple_of(i * DP, DP), DP), :] = o.astype(bf16)

    def attend(use_max):
        def head(i, carry):
            grp = pl.multiple_of(((i % H) // 4) * 128, 128)
            s = jax.lax.dot_general(k_s[i // H, :, pl.ds(grp, 128)], qm_s[...], NN,
                                    preferred_element_type=f32)
            finalize(jnp.where(i == 0, 2 * H, i - 1))
            if use_max:
                s = s - jnp.max(s, axis=0, keepdims=True)
            p = jnp.exp2(s).astype(bf16)
            vT = vT_s[pl.ds(pl.multiple_of(i * DP, DP), DP), :]
            acc = jax.lax.dot_general(vT, p, NN, preferred_element_type=f32)
            masked_q(jnp.minimum(i + 1, 2 * H - 1))
            acc_s[...] = acc
            return carry
        jax.lax.fori_loop(0, 2 * H, head, 0)

    masked_q(jnp.int32(0))
    acc_s[...] = jnp.ones((DP, S), f32)

    @pl.when(safe)
    def _fast():
        attend(False)

    @pl.when(jnp.logical_not(safe))
    def _exact_max():
        attend(True)

    finalize(jnp.int32(2 * H - 1))

    out_cp = []
    for c, (c0, n) in enumerate(OUT_CHUNKS):
        cols = pl.ds(c0, n)
        o = oT_s[0:2 * HP, cols].astype(f32)
        o = jnp.concatenate([o[i * DP:i * DP + DH, :] for i in range(2 * H)], axis=0).astype(bf16)
        outT = jax.lax.dot_general(woT_s[...], o, NN, preferred_element_type=f32)
        out_buf[:, cols] = outT.astype(bf16)
        cp = pltpu.make_async_copy(out_buf.at[:, cols], out_hbm.at[:, cols], out_sems.at[c])
        cp.start()
        out_cp.append(cp)
    for cp in out_cp:
        cp.wait()


def _reduce(fn, xs):
    acc = xs[0]
    for x in xs[1:]:
        acc = fn(acc, x)
    return acc


@jax.jit
def pallas_gated_mix__mha_block__mha_block__prompt_kernel(
    A_x: jax.Array,
    A_wqkv: jax.Array,
    A_wo: jax.Array,
    B_x: jax.Array,
    B_wqkv: jax.Array,
    B_wo: jax.Array,
    gate_w: jax.Array,
):
    del B_x
    hbm = pl.BlockSpec(memory_space=pltpu.HBM)
    outT = pl.pallas_call(
        _kernel,
        in_specs=[hbm] * 6,
        out_specs=hbm,
        out_shape=jax.ShapeDtypeStruct((D, S), bf16),
        scratch_shapes=[
            pltpu.VMEM((D,), bf16),
            pltpu.VMEM((D, S), bf16),
            pltpu.VMEM((S, D), bf16),
            pltpu.VMEM((2, D, 3 * D), bf16),
            pltpu.VMEM((2 * D, D), bf16),
            pltpu.VMEM((2, 3 * D, D), f32),
            pltpu.VMEM((2, 2 * D, D), bf16),
            pltpu.VMEM((2, HP, D), bf16),
            pltpu.VMEM((2, S, HP), bf16),
            pltpu.VMEM((2 * HP, S), bf16),
            pltpu.VMEM((2 * HP, S), bf16),
            pltpu.VMEM((D, 2 * D), bf16),
            pltpu.VMEM((2 * HP + DP, S), bf16),
            pltpu.VMEM((128, S), bf16),
            pltpu.VMEM((DP, S), f32),
            pltpu.VMEM((8, S), f32),
            pltpu.VMEM((D, S), bf16),
            pltpu.SemaphoreType.DMA((NC + 4,)),
            pltpu.SemaphoreType.DMA((len(OUT_CHUNKS),)),
            pltpu.SemaphoreType.DMA((3,)),
        ],
        compiler_params=pltpu.CompilerParams(vmem_limit_bytes=100 * 1024 * 1024),
    )(A_x.reshape(S, D).T, A_wqkv, A_wo, B_wqkv, B_wo, gate_w)
    return outT.T.reshape(1, S, D)
```
